```python
import jax
import jax.numpy as jnp

def _softmax(x, axis=-1):
    return jax.nn.softmax(x, axis=axis)
def _gelu(x):
    return jax.nn.gelu(x, approximate=True)
def _silu(x):
    return jax.nn.silu(x)
def _sigmoid(x):
    return jax.nn.sigmoid(x)
def _layernorm(x, axis=-1, eps=1e-5):
    m = jnp.mean(x, axis=axis, keepdims=True)
    v = jnp.var(x, axis=axis, keepdims=True)
    return (x - m) / jnp.sqrt(v + eps)
def _scatter_add(tgt, idx, src, axis=0):
    return tgt.at[idx].add(src)
def _segment_sum(src, seg, n):
    return jax.ops.segment_sum(src, seg, n)
class _Rng:
    def __init__(self, key):
        self._k = key
    def _next(self):
        self._k, sub = jax.random.split(self._k)
        return sub
    def normal(self, shape):
        return jax.random.normal(self._next(), shape, dtype=jnp.bfloat16)
    def randint(self, lo, hi, shape):
        return jax.random.randint(self._next(), shape, lo, hi, dtype=jnp.int32)
    def uniform(self, shape, lo=0.0, hi=1.0):
        return jax.random.uniform(self._next(), shape, jnp.bfloat16, lo, hi)
    def permutation(self, n):
        return jax.random.permutation(self._next(), n)


kernel_name = 'parallel_sum__sliding_block_cached__moe_arch_mod__decode'

def setup_inputs():
    _rng = _Rng(jax.random.key(int.from_bytes(__import__("os").urandom(4), "little")))
    _w = (lambda a: (lambda t: t.astype(jnp.bfloat16) if jnp.issubdtype(t.dtype, jnp.floating) else t)(jnp.asarray(a)))
    def _A_setup():
        B, Sq, D = 1, 1, 512
        Hq, Hkv, Sk, Dh = 32, 8, 65536, 128
        assert Hq % Hkv == 0, (Hq, Hkv)
        return {
            "x": _w((lambda *s: _rng.normal(s) * 0.05)(B, Sq, D)),
            "k_cache": _w((lambda *s: _rng.normal(s) * 0.05)(B, Hkv, Sk, Dh)),
            "v_cache": _w((lambda *s: _rng.normal(s) * 0.05)(B, Hkv, Sk, Dh)),
            "wq": _w((lambda *s: _rng.normal(s) * 0.05)(D, Hq * Dh) * (D ** -0.5)),
            "wo": _w((lambda *s: _rng.normal(s) * 0.05)(Hq * Dh, D) * ((Hq * Dh) ** -0.5)),
        }
    _A_in = _A_setup()

    def _B_setup():
        B, S, D, F, C = 1, 1, 512, 1792, 1
        return {
            "x": _w((lambda *s: _rng.normal(s) * 0.05)(B, S, D)),
            "w_r": _w((lambda *s: _rng.normal(s) * 0.05)(D)),
            "w_gate": _w((lambda *s: _rng.normal(s) * 0.05)(D, F)),
            "w_up": _w((lambda *s: _rng.normal(s) * 0.05)(D, F)),
            "w_down": _w((lambda *s: _rng.normal(s) * 0.05)(F, D)),
        }
    _B_in = _B_setup()

    return {
        "A_x": _A_in["x"],
        "A_k_cache": _A_in["k_cache"],
        "A_v_cache": _A_in["v_cache"],
        "A_wq": _A_in["wq"],
        "A_wo": _A_in["wo"],
        "B_x": _B_in["x"],
        "B_w_r": _B_in["w_r"],
        "B_w_gate": _B_in["w_gate"],
        "B_w_up": _B_in["w_up"],
        "B_w_down": _B_in["w_down"],
    }

def reference(A_x, A_k_cache, A_v_cache, A_wq, A_wo, B_x, B_w_r, B_w_gate, B_w_up, B_w_down):
    def _A_ref(x, k_cache, v_cache, wq, wo):
        B, Sq, D = x.shape
        Hq, Dh = 32, 128
        Hkv, Sk = k_cache.shape[1], k_cache.shape[2]
        W = min(4096, max(256, Sk // 4))
        rep = Hq // Hkv
        q = (lambda x, *d: x.transpose(*d))((x @ wq).reshape(B, Sq, Hq, Dh), 0, 2, 1, 3)
        k = jnp.repeat(k_cache[:, :, Sk - W:, :], rep, axis=1)
        v = jnp.repeat(v_cache[:, :, Sk - W:, :], rep, axis=1)
        scores = jnp.einsum("bhqd,bhkd->bhqk", q, k) * (Dh ** -0.5)
        p = _softmax(scores, axis=-1)
        o = jnp.einsum("bhqk,bhkd->bhqd", p, v)
        return (lambda x, *d: x.transpose(*d))(o, 0, 2, 1, 3).reshape(B, Sq, Hq * Dh) @ wo

    def _B_ref(x, w_r, w_gate, w_up, w_down):
        B, S, D = x.shape
        C = 1
        r = x @ w_r
        idx = jnp.argsort(-r, axis=-1)[:, :C]
        idx_e = jnp.repeat(idx.reshape(B, C, 1), D, axis=2)
        x_sel = jnp.take_along_axis(x, idx_e, axis=1)
        g = _silu(x_sel @ w_gate)
        u = x_sel @ w_up
        y = (g * u) @ w_down
        r_sel = _sigmoid(jnp.take_along_axis(r, idx, axis=1))
        y = y * r_sel.reshape(B, C, 1)
        b_off = (jnp.arange(B) * S).reshape(B, 1)
        flat_idx = (idx + b_off).reshape(B * C)
        zero = (x * 0.0).reshape(B * S, D)
        upd = _scatter_add(zero, flat_idx, y.reshape(B * C, D), axis=0)
        return x + upd.reshape(B, S, D)

    x = A_x
    xn = _layernorm(x, axis=-1)
    return x + _A_ref(xn, A_k_cache, A_v_cache, A_wq, A_wo) + _B_ref(xn, B_w_r, B_w_gate, B_w_up, B_w_down)
```

```python
import jax
import jax.numpy as jnp
from jax import lax
import jax.experimental.pallas as pl
import jax.experimental.pallas.tpu as pltpu

_HQ = 32
_DH = 128
_LN_EPS = 1e-5
_WINDOW = 4
_CHUNK_BYTES = 1 << 20
_LANES = 128
_SUBLANES = 8


def _row_chunks(n_rows, rows_per_chunk):
    return [(s, min(rows_per_chunk, n_rows - s)) for s in range(0, n_rows, rows_per_chunk)]


@jax.jit
def pallas_parallel_sum__sliding_block_cached__moe_arch_mod__decode_kernel(
A_x: jax.Array,
    A_k_cache: jax.Array,
    A_v_cache: jax.Array,
    A_wq: jax.Array,
    A_wo: jax.Array,
    B_x: jax.Array,
    B_w_r: jax.Array,
    B_w_gate: jax.Array,
    B_w_up: jax.Array,
    B_w_down: jax.Array,
):
    del B_x
    f32 = jnp.float32
    cdt = A_x.dtype

    batch, s_q, d_model = A_x.shape
    _, n_kv, s_k, d_head = A_k_cache.shape
    d_ffn = B_w_gate.shape[1]
    assert batch == 1 and s_q == 1 and d_head == _DH and _HQ % n_kv == 0
    assert A_wq.shape == (d_model, _HQ * _DH) and A_wo.shape == (_HQ * _DH, d_model)
    assert B_w_gate.shape == B_w_up.shape == (d_model, d_ffn)
    assert B_w_down.shape == (d_ffn, d_model) and B_w_r.shape == (d_model,)
    win = min(4096, max(256, s_k // 4))
    rep = _HQ // n_kv
    assert rep <= _SUBLANES and _SUBLANES % rep == 0
    assert d_model % (2 * _LANES) == 0 and win % _LANES == 0 and d_ffn % _LANES == 0
    group_w = rep * _DH
    sm_scale = _DH ** -0.5
    itemsize = jnp.dtype(cdt).itemsize

    def rows_for(row_bytes):
        return max(_LANES, _CHUNK_BYTES // row_bytes // _LANES * _LANES)

    wq_chunks = _row_chunks(d_model, rows_for(_HQ * _DH * itemsize))
    wgu_chunks = _row_chunks(d_model, d_model // 2)
    wo_chunks = _row_chunks(_HQ * _DH, rows_for(d_model * itemsize))
    wd_vpu_rows = (128, 64, 64)
    wd_mxu_total = d_ffn - sum(wd_vpu_rows)
    assert wd_mxu_total >= 0
    wd_mxu_rows = []
    left = wd_mxu_total
    while left > 0:
        step = min(left, 512 if left > 512 else 256)
        wd_mxu_rows.append(step)
        left -= step
    wd_chunks, s = [], 0
    for r in (*wd_mxu_rows, *wd_vpu_rows):
        wd_chunks.append((s, r))
        s += r
    n_wd_mxu = len(wd_mxu_rows)

    def body(x_hbm, k_hbm, v_hbm, wq_hbm, wo_hbm, wr_hbm, wg_hbm, wu_hbm, wd_hbm, out_hbm,
             x_v, wr_v, k_v, v_v, wq_v, wo_v, wg_v, wu_v, wd_v, out_v, out_sem, sems):
        stream = []

        def enqueue(src, dst):
            stream.append(pltpu.make_async_copy(src, dst, sems.at[len(stream) % _WINDOW]))

        for s0, n in wq_chunks:
            enqueue(wq_hbm.at[pl.ds(s0, n)], wq_v.at[pl.ds(s0, n)])
        for h in range(n_kv):
            enqueue(k_hbm.at[0, h, pl.ds(s_k - win, win)], k_v.at[h])
            enqueue(v_hbm.at[0, h, pl.ds(s_k - win, win)], v_v.at[h])
        for s0, n in wgu_chunks:
            enqueue(wg_hbm.at[pl.ds(s0, n)], wg_v.at[pl.ds(s0, n)])
        for s0, n in wgu_chunks:
            enqueue(wu_hbm.at[pl.ds(s0, n)], wu_v.at[pl.ds(s0, n)])
        for s0, n in wo_chunks:
            enqueue(wo_hbm.at[pl.ds(s0, n)], wo_v.at[pl.ds(s0, n)])
        for s0, n in wd_chunks:
            enqueue(wd_hbm.at[pl.ds(s0, n)], wd_v.at[pl.ds(s0, n)])
        started, waited = [0], [0]

        def start_upto(n_started):
            while started[0] < min(n_started, len(stream)):
                stream[started[0]].start()
                started[0] += 1

        def next_chunk():
            stream[waited[0]].wait()
            waited[0] += 1
            start_upto(waited[0] + _WINDOW)

        x_copy = pltpu.make_async_copy(x_hbm, x_v, sems.at[_WINDOW - 1])
        wr_copy = pltpu.make_async_copy(wr_hbm, wr_v, sems.at[_WINDOW - 1])
        start_upto(1)
        x_copy.start()
        wr_copy.start()
        start_upto(_WINDOW - 1)
        x_copy.wait()
        wr_copy.wait()
        start_upto(_WINDOW)

        row = lax.broadcasted_iota(jnp.int32, (_SUBLANES, _DH), 0)

        x = x_v[0].astype(f32)
        mean = jnp.mean(x, axis=-1, keepdims=True)
        xc = x - mean
        var = jnp.mean(xc * xc, axis=-1, keepdims=True)
        xn = xc / jnp.sqrt(var + _LN_EPS)
        xn_c = xn.astype(cdt)
        r = jnp.sum(xn_c.astype(f32) * wr_v[...].astype(f32).reshape(1, d_model),
                    axis=-1, keepdims=True)
        gate_r = jax.nn.sigmoid(r)
        x_rows = jnp.broadcast_to(xn_c, (_SUBLANES, d_model))

        q = jnp.zeros((_SUBLANES, _HQ * _DH), f32)
        for s0, n in wq_chunks:
            next_chunk()
            q = q + jnp.dot(x_rows[:, s0:s0 + n], wq_v[pl.ds(s0, n), :],
                            preferred_element_type=f32)
        q = q.astype(cdt)

        o_rows = []
        for h in range(n_kv):
            q_h = q[:, h * group_w:h * group_w + _DH]
            for j in range(1, rep):
                q_h = jnp.where(row % rep == j,
                                q[:, h * group_w + j * _DH:h * group_w + (j + 1) * _DH], q_h)
            next_chunk()
            sc = lax.dot_general(q_h, k_v[h], (((1,), (1,)), ((), ())),
                                 preferred_element_type=f32) * sm_scale
            p = jnp.exp(sc - jnp.max(sc, axis=-1, keepdims=True))
            denom = jnp.sum(p, axis=-1, keepdims=True)
            next_chunk()
            o = jnp.dot(p.astype(cdt), v_v[h], preferred_element_type=f32) / denom
            o = o.astype(cdt)
            o_rows += [jnp.where(row == j, o, jnp.zeros_like(o)) for j in range(rep)]

        def up_proj(w_v):
            acc = jnp.zeros((_SUBLANES, d_ffn), f32)
            for s0, n in wgu_chunks:
                next_chunk()
                acc = acc + jnp.dot(x_rows[:, s0:s0 + n], w_v[pl.ds(s0, n), :],
                                    preferred_element_type=f32)
            return acc

        g = up_proj(wg_v)
        u = up_proj(wu_v)
        hid = (jax.nn.silu(g) * u).astype(cdt)

        hid_col = []
        for c0 in range(wd_mxu_total, d_ffn, _LANES):
            piece = hid[0:1, c0:c0 + _LANES].astype(f32) * gate_r
            hid_col.append(jnp.broadcast_to(piece, (_LANES, _LANES)).T)
        hid_col = jnp.concatenate(hid_col, axis=0)

        attn = jnp.zeros((_SUBLANES, d_model), f32)
        for s0, n in wo_chunks:
            next_chunk()
            lhs = jnp.concatenate(o_rows[s0 // _DH:(s0 + n) // _DH], axis=1)
            attn = attn + jnp.dot(lhs, wo_v[pl.ds(s0, n), :], preferred_element_type=f32)
        base = x + jnp.sum(attn, axis=0, keepdims=True) + (xn + xn * 0.0)

        y = jnp.zeros((_SUBLANES, d_model), f32)
        for s0, n in wd_chunks[:n_wd_mxu]:
            next_chunk()
            y = y + jnp.dot(hid[:, s0:s0 + n], wd_v[pl.ds(s0, n), :],
                            preferred_element_type=f32)
        row_d = lax.broadcasted_iota(jnp.int32, (_SUBLANES, d_model), 0)
        part = jnp.where(row_d == 0, base + y * gate_r, 0.0)
        for s0, n in wd_chunks[n_wd_mxu:]:
            next_chunk()
            w = wd_v[pl.ds(s0, n), :].astype(f32)
            hc = hid_col[s0 - wd_mxu_total:s0 - wd_mxu_total + n, :]
            prod = w * jnp.concatenate([hc] * (d_model // _LANES), axis=1)
            part = part + prod.reshape(n // _SUBLANES, _SUBLANES, d_model).sum(axis=0)
        assert waited[0] == started[0] == len(stream)

        out_v[0] = jnp.sum(part, axis=0, keepdims=True).astype(out_v.dtype)
        pltpu.make_async_copy(out_v, out_hbm, out_sem.at[0]).start()

    def kernel_function(*refs):
        pl.run_scoped(lambda sems: body(*refs, sems), pltpu.SemaphoreType.DMA((_WINDOW,)))
        out_hbm, out_v, out_sem = refs[9], refs[-2], refs[-1]
        pltpu.make_async_copy(out_v, out_hbm, out_sem.at[0]).wait()

    hbm = pl.BlockSpec(memory_space=pl.ANY)
    return pl.pallas_call(
        kernel_function,
        out_shape=jax.ShapeDtypeStruct(A_x.shape, cdt),
        in_specs=[hbm] * 9,
        out_specs=hbm,
        scratch_shapes=[
            pltpu.VMEM(A_x.shape, cdt),
            pltpu.VMEM(B_w_r.shape, B_w_r.dtype),
            pltpu.VMEM((n_kv, win, _DH), A_k_cache.dtype),
            pltpu.VMEM((n_kv, win, _DH), A_v_cache.dtype),
            pltpu.VMEM(A_wq.shape, A_wq.dtype),
            pltpu.VMEM(A_wo.shape, A_wo.dtype),
            pltpu.VMEM(B_w_gate.shape, B_w_gate.dtype),
            pltpu.VMEM(B_w_up.shape, B_w_up.dtype),
            pltpu.VMEM(B_w_down.shape, B_w_down.dtype),
            pltpu.VMEM(A_x.shape, cdt),
            pltpu.SemaphoreType.DMA((1,)),
        ],
        compiler_params=pltpu.CompilerParams(vmem_limit_bytes=48 << 20),
        name="psum_swa_mod_decode",
    )(A_x, A_k_cache, A_v_cache, A_wq, A_wo, B_w_r, B_w_gate, B_w_up, B_w_down)
```

```python
import jax
import jax.numpy as jnp
from jax import lax
import jax.experimental.pallas as pl
import jax.experimental.pallas.tpu as pltpu

_HQ = 32
_DH = 128
_LN_EPS = 1e-5
_WINDOW = 4
_CHUNK_BYTES = 1 << 20
_LANES = 128
_SUBLANES = 8


def _row_chunks(n_rows, rows_per_chunk):
    return [(s, min(rows_per_chunk, n_rows - s)) for s in range(0, n_rows, rows_per_chunk)]


@jax.jit
def pallas_parallel_sum__sliding_block_cached__moe_arch_mod__decode_kernel(
A_x: jax.Array,
    A_k_cache: jax.Array,
    A_v_cache: jax.Array,
    A_wq: jax.Array,
    A_wo: jax.Array,
    B_x: jax.Array,
    B_w_r: jax.Array,
    B_w_gate: jax.Array,
    B_w_up: jax.Array,
    B_w_down: jax.Array,
):
    del B_x
    f32 = jnp.float32
    cdt = A_x.dtype

    batch, s_q, d_model = A_x.shape
    _, n_kv, s_k, d_head = A_k_cache.shape
    d_ffn = B_w_gate.shape[1]
    assert batch == 1 and s_q == 1 and d_head == _DH and _HQ % n_kv == 0
    assert A_wq.shape == (d_model, _HQ * _DH) and A_wo.shape == (_HQ * _DH, d_model)
    assert B_w_gate.shape == B_w_up.shape == (d_model, d_ffn)
    assert B_w_down.shape == (d_ffn, d_model) and B_w_r.shape == (d_model,)
    win = min(4096, max(256, s_k // 4))
    rep = _HQ // n_kv
    assert rep <= _SUBLANES and _SUBLANES % rep == 0
    assert d_model % (2 * _LANES) == 0 and win % _LANES == 0 and d_ffn % _LANES == 0
    group_w = rep * _DH
    sm_scale = _DH ** -0.5
    itemsize = jnp.dtype(cdt).itemsize

    def rows_for(row_bytes):
        return max(_LANES, _CHUNK_BYTES // row_bytes // _LANES * _LANES)

    wq_chunks = _row_chunks(d_model, rows_for(_HQ * _DH * itemsize))
    wgu_chunks = _row_chunks(d_model, d_model // 2)
    wo_chunks = _row_chunks(_HQ * _DH, rows_for(d_model * itemsize))
    wd_vpu_rows = (128, 64, 64)
    wd_mxu_total = d_ffn - sum(wd_vpu_rows)
    assert wd_mxu_total >= 0
    wd_mxu_rows = []
    left = wd_mxu_total
    while left > 0:
        step = min(left, 512 if left > 512 else 256)
        wd_mxu_rows.append(step)
        left -= step
    wd_chunks, s = [], 0
    for r in (*wd_mxu_rows, *wd_vpu_rows):
        wd_chunks.append((s, r))
        s += r
    n_wd_mxu = len(wd_mxu_rows)

    def body(x_hbm, k_hbm, v_hbm, wq_hbm, wo_hbm, wr_hbm, wg_hbm, wu_hbm, wd_hbm, out_hbm,
             x_v, wr_v, k_v, v_v, wq_v, wo_v, wg_v, wu_v, wd_v, out_v, sems, out_sem):
        stream = []

        def enqueue(src, dst):
            stream.append(pltpu.make_async_copy(src, dst, sems.at[len(stream) % _WINDOW]))

        for s0, n in wq_chunks:
            enqueue(wq_hbm.at[pl.ds(s0, n)], wq_v.at[pl.ds(s0, n)])
        for h in range(n_kv):
            enqueue(k_hbm.at[0, h, pl.ds(s_k - win, win)], k_v.at[h])
            enqueue(v_hbm.at[0, h, pl.ds(s_k - win, win)], v_v.at[h])
        for s0, n in wgu_chunks:
            enqueue(wg_hbm.at[pl.ds(s0, n)], wg_v.at[pl.ds(s0, n)])
        for s0, n in wgu_chunks:
            enqueue(wu_hbm.at[pl.ds(s0, n)], wu_v.at[pl.ds(s0, n)])
        for s0, n in wo_chunks:
            enqueue(wo_hbm.at[pl.ds(s0, n)], wo_v.at[pl.ds(s0, n)])
        for s0, n in wd_chunks:
            enqueue(wd_hbm.at[pl.ds(s0, n)], wd_v.at[pl.ds(s0, n)])
        started, waited = [0], [0]

        def start_upto(n_started):
            while started[0] < min(n_started, len(stream)):
                stream[started[0]].start()
                started[0] += 1

        def next_chunk():
            stream[waited[0]].wait()
            waited[0] += 1
            start_upto(waited[0] + _WINDOW)

        x_copy = pltpu.make_async_copy(x_hbm, x_v, sems.at[_WINDOW - 1])
        wr_copy = pltpu.make_async_copy(wr_hbm, wr_v, sems.at[_WINDOW - 1])
        start_upto(1)
        x_copy.start()
        wr_copy.start()
        start_upto(_WINDOW - 1)
        x_copy.wait()
        wr_copy.wait()
        start_upto(_WINDOW)

        row = lax.broadcasted_iota(jnp.int32, (_SUBLANES, _DH), 0)

        x = x_v[0].astype(f32)
        mean = jnp.mean(x, axis=-1, keepdims=True)
        xc = x - mean
        var = jnp.mean(xc * xc, axis=-1, keepdims=True)
        xn = xc / jnp.sqrt(var + _LN_EPS)
        xn_c = xn.astype(cdt)
        r = jnp.sum(xn_c.astype(f32) * wr_v[...].astype(f32).reshape(1, d_model),
                    axis=-1, keepdims=True)
        gate_r = jax.nn.sigmoid(r)
        x_rows = jnp.broadcast_to(xn_c, (_SUBLANES, d_model))

        q = jnp.zeros((_SUBLANES, _HQ * _DH), f32)
        for s0, n in wq_chunks:
            next_chunk()
            q = q + jnp.dot(x_rows[:, s0:s0 + n], wq_v[pl.ds(s0, n), :],
                            preferred_element_type=f32)
        q = q.astype(cdt)

        o_rows = []
        for h in range(n_kv):
            q_h = q[:, h * group_w:h * group_w + _DH]
            for j in range(1, rep):
                q_h = jnp.where(row % rep == j,
                                q[:, h * group_w + j * _DH:h * group_w + (j + 1) * _DH], q_h)
            next_chunk()
            sc = lax.dot_general(q_h, k_v[h], (((1,), (1,)), ((), ())),
                                 preferred_element_type=f32) * sm_scale
            p = jnp.exp(sc - jnp.max(sc, axis=-1, keepdims=True))
            denom = jnp.sum(p, axis=-1, keepdims=True)
            next_chunk()
            o = jnp.dot(p.astype(cdt), v_v[h], preferred_element_type=f32) / denom
            o = o.astype(cdt)
            o_rows += [jnp.where(row == j, o, jnp.zeros_like(o)) for j in range(rep)]

        def up_proj(w_v):
            acc = jnp.zeros((_SUBLANES, d_ffn), f32)
            for s0, n in wgu_chunks:
                next_chunk()
                acc = acc + jnp.dot(x_rows[:, s0:s0 + n], w_v[pl.ds(s0, n), :],
                                    preferred_element_type=f32)
            return acc

        g = up_proj(wg_v)
        u = up_proj(wu_v)
        hid = (jax.nn.silu(g) * u).astype(cdt)

        hid_col = []
        for c0 in range(wd_mxu_total, d_ffn, _LANES):
            piece = hid[0:1, c0:c0 + _LANES].astype(f32) * gate_r
            hid_col.append(jnp.broadcast_to(piece, (_LANES, _LANES)).T)
        hid_col = jnp.concatenate(hid_col, axis=0)

        attn = jnp.zeros((_SUBLANES, d_model), f32)
        for s0, n in wo_chunks:
            next_chunk()
            lhs = jnp.concatenate(o_rows[s0 // _DH:(s0 + n) // _DH], axis=1)
            attn = attn + jnp.dot(lhs, wo_v[pl.ds(s0, n), :], preferred_element_type=f32)
        base = x + jnp.sum(attn, axis=0, keepdims=True) + (xn + xn * 0.0)

        y = jnp.zeros((_SUBLANES, d_model), f32)
        for s0, n in wd_chunks[:n_wd_mxu]:
            next_chunk()
            y = y + jnp.dot(hid[:, s0:s0 + n], wd_v[pl.ds(s0, n), :],
                            preferred_element_type=f32)
        row_d = lax.broadcasted_iota(jnp.int32, (_SUBLANES, d_model), 0)
        part = jnp.where(row_d == 0, base + y * gate_r, 0.0)
        for s0, n in wd_chunks[n_wd_mxu:]:
            next_chunk()
            w = wd_v[pl.ds(s0, n), :].astype(f32)
            hc = hid_col[s0 - wd_mxu_total:s0 - wd_mxu_total + n, :]
            prod = w * jnp.concatenate([hc] * (d_model // _LANES), axis=1)
            part = part + prod.reshape(n // _SUBLANES, _SUBLANES, d_model).sum(axis=0)
        assert waited[0] == started[0] == len(stream)

        out_v[0] = jnp.sum(part, axis=0, keepdims=True).astype(out_v.dtype)
        out_copy = pltpu.make_async_copy(out_v, out_hbm, out_sem.at[0])
        out_copy.start()
        out_copy.wait()

    def kernel_function(*refs):
        pl.run_scoped(lambda sems, out_sem: body(*refs, sems, out_sem),
                      pltpu.SemaphoreType.DMA((_WINDOW,)), pltpu.SemaphoreType.DMA((1,)))

    hbm = pl.BlockSpec(memory_space=pl.ANY)
    return pl.pallas_call(
        kernel_function,
        out_shape=jax.ShapeDtypeStruct(A_x.shape, cdt),
        in_specs=[hbm] * 9,
        out_specs=hbm,
        scratch_shapes=[
            pltpu.VMEM(A_x.shape, cdt),
            pltpu.VMEM(B_w_r.shape, B_w_r.dtype),
            pltpu.VMEM((n_kv, win, _DH), A_k_cache.dtype),
            pltpu.VMEM((n_kv, win, _DH), A_v_cache.dtype),
            pltpu.VMEM(A_wq.shape, A_wq.dtype),
            pltpu.VMEM(A_wo.shape, A_wo.dtype),
            pltpu.VMEM(B_w_gate.shape, B_w_gate.dtype),
            pltpu.VMEM(B_w_up.shape, B_w_up.dtype),
            pltpu.VMEM(B_w_down.shape, B_w_down.dtype),
            pltpu.VMEM(A_x.shape, cdt),
        ],
        compiler_params=pltpu.CompilerParams(vmem_limit_bytes=48 << 20),
        name="psum_swa_mod_decode",
    )(A_x, A_k_cache, A_v_cache, A_wq, A_wo, B_w_r, B_w_gate, B_w_up, B_w_down)
```

```python
import jax
import jax.numpy as jnp
from jax import lax
import jax.experimental.pallas as pl
import jax.experimental.pallas.tpu as pltpu

_HQ = 32
_DH = 128
_LN_EPS = 1e-5
_CHUNK_BYTES = 1 << 20
_PIECE_BYTES = 32 << 10
_AHEAD_BYTES = 4 << 20
_NUM_SEMS = 8
_PRIORITIES = (0, 1, 1)
_LANES = 128
_SUBLANES = 8


def _row_chunks(n_rows, rows_per_chunk):
    return [(s, min(rows_per_chunk, n_rows - s)) for s in range(0, n_rows, rows_per_chunk)]


@jax.jit
def pallas_parallel_sum__sliding_block_cached__moe_arch_mod__decode_kernel(
A_x: jax.Array,
    A_k_cache: jax.Array,
    A_v_cache: jax.Array,
    A_wq: jax.Array,
    A_wo: jax.Array,
    B_x: jax.Array,
    B_w_r: jax.Array,
    B_w_gate: jax.Array,
    B_w_up: jax.Array,
    B_w_down: jax.Array,
):
    del B_x
    f32 = jnp.float32
    cdt = A_x.dtype

    batch, s_q, d_model = A_x.shape
    _, n_kv, s_k, d_head = A_k_cache.shape
    d_ffn = B_w_gate.shape[1]
    assert batch == 1 and s_q == 1 and d_head == _DH and _HQ % n_kv == 0
    assert A_wq.shape == (d_model, _HQ * _DH) and A_wo.shape == (_HQ * _DH, d_model)
    assert B_w_gate.shape == B_w_up.shape == (d_model, d_ffn)
    assert B_w_down.shape == (d_ffn, d_model) and B_w_r.shape == (d_model,)
    win = min(4096, max(256, s_k // 4))
    rep = _HQ // n_kv
    assert rep <= _SUBLANES and _SUBLANES % rep == 0
    assert d_model % (2 * _LANES) == 0 and win % _LANES == 0 and d_ffn % _LANES == 0
    group_w = rep * _DH
    sm_scale = _DH ** -0.5
    itemsize = jnp.dtype(cdt).itemsize

    def rows_for(row_bytes):
        return max(_LANES, _CHUNK_BYTES // row_bytes // _LANES * _LANES)

    wq_chunks = _row_chunks(d_model, rows_for(_HQ * _DH * itemsize))
    wgu_chunks = _row_chunks(d_model, d_model // 2)
    wo_chunks = _row_chunks(_HQ * _DH, rows_for(d_model * itemsize))
    wd_vpu_rows = (128, 64, 32, 32)
    wd_mxu_total = d_ffn - sum(wd_vpu_rows)
    assert wd_mxu_total >= 0
    wd_mxu_rows = []
    left = wd_mxu_total
    while left > 0:
        step = min(left, 512 if left > 512 else 256)
        wd_mxu_rows.append(step)
        left -= step
    wd_chunks, s = [], 0
    for r in (*wd_mxu_rows, *wd_vpu_rows):
        wd_chunks.append((s, r))
        s += r
    n_wd_mxu = len(wd_mxu_rows)

    def body(x_hbm, k_hbm, v_hbm, wq_hbm, wo_hbm, wr_hbm, wg_hbm, wu_hbm, wd_hbm, out_hbm,
             x_v, wr_v, k_v, v_v, wq_v, wo_v, wg_v, wu_v, wd_v, out_v, sems, small_sems, out_sem):
        stream = []

        def enqueue(src, dst, n_rows, n_cols):
            row_bytes = n_cols * itemsize
            if 2 * row_bytes * _SUBLANES > 3 * _PIECE_BYTES:
                p_rows = _SUBLANES
                p_cols = max(_LANES, _PIECE_BYTES // (p_rows * itemsize) // _LANES * _LANES)
            else:
                p_rows = max(_SUBLANES, _PIECE_BYTES // row_bytes // _SUBLANES * _SUBLANES)
                p_cols = n_cols
            sem = sems.at[len(stream) % _NUM_SEMS]
            pieces = []
            for r in range(0, n_rows, p_rows):
                for c in range(0, n_cols, p_cols):
                    rows, cols = pl.ds(r, min(p_rows, n_rows - r)), pl.ds(c, min(p_cols, n_cols - c))
                    if p_cols >= n_cols:
                        pieces.append(pltpu.make_async_copy(src.at[rows], dst.at[rows], sem))
                    else:
                        pieces.append(pltpu.make_async_copy(src.at[rows, cols], dst.at[rows, cols], sem))
            n_pat0 = _PRIORITIES.count(0)
            n0 = (len(pieces) * n_pat0 + len(_PRIORITIES) // 2) // len(_PRIORITIES)
            n0 = min(max(n0, 1), max(len(pieces) - 1, 1))
            todo = {0: pieces[:n0], 1: pieces[n0:]}
            issue, k = [], 0
            while todo[0] or todo[1]:
                prio = _PRIORITIES[k % len(_PRIORITIES)]
                k += 1
                if todo[prio]:
                    issue.append((todo[prio].pop(0), prio))
            stream.append((pltpu.make_async_copy(dst, dst, sem), issue, n_rows * row_bytes))

        for s0, n in wq_chunks:
            enqueue(wq_hbm.at[pl.ds(s0, n)], wq_v.at[pl.ds(s0, n)], n, _HQ * _DH)
        for h in range(n_kv):
            enqueue(k_hbm.at[0, h, pl.ds(s_k - win, win)], k_v.at[h], win, _DH)
            enqueue(v_hbm.at[0, h, pl.ds(s_k - win, win)], v_v.at[h], win, _DH)
        for s0, n in wgu_chunks:
            enqueue(wg_hbm.at[pl.ds(s0, n)], wg_v.at[pl.ds(s0, n)], n, d_ffn)
        for s0, n in wgu_chunks:
            enqueue(wu_hbm.at[pl.ds(s0, n)], wu_v.at[pl.ds(s0, n)], n, d_ffn)
        for s0, n in wo_chunks:
            enqueue(wo_hbm.at[pl.ds(s0, n)], wo_v.at[pl.ds(s0, n)], n, d_model)
        for s0, n in wd_chunks:
            enqueue(wd_hbm.at[pl.ds(s0, n)], wd_v.at[pl.ds(s0, n)], n, d_model)
        started, waited = [0], [0]

        def top_up():
            while (started[0] < len(stream) and started[0] - waited[0] < _NUM_SEMS
                   and sum(c[2] for c in stream[waited[0]:started[0]]) < _AHEAD_BYTES):
                for copy, prio in stream[started[0]][1]:
                    copy.start(priority=prio)
                started[0] += 1

        def next_chunk():
            stream[waited[0]][0].wait()
            waited[0] += 1
            top_up()

        x_copy = pltpu.make_async_copy(x_hbm, x_v, small_sems.at[0])
        wr_copy = pltpu.make_async_copy(wr_hbm, wr_v, small_sems.at[1])
        x_copy.start()
        wr_copy.start()
        top_up()
        x_copy.wait()
        wr_copy.wait()

        row = lax.broadcasted_iota(jnp.int32, (_SUBLANES, _DH), 0)

        x = x_v[0].astype(f32)
        mean = jnp.mean(x, axis=-1, keepdims=True)
        xc = x - mean
        var = jnp.mean(xc * xc, axis=-1, keepdims=True)
        xn = xc / jnp.sqrt(var + _LN_EPS)
        xn_c = xn.astype(cdt)
        r = jnp.sum(xn_c.astype(f32) * wr_v[...].astype(f32).reshape(1, d_model),
                    axis=-1, keepdims=True)
        gate_r = jax.nn.sigmoid(r)
        x_rows = jnp.broadcast_to(xn_c, (_SUBLANES, d_model))

        q = jnp.zeros((_SUBLANES, _HQ * _DH), f32)
        for s0, n in wq_chunks:
            next_chunk()
            q = q + jnp.dot(x_rows[:, s0:s0 + n], wq_v[pl.ds(s0, n), :],
                            preferred_element_type=f32)
        q = q.astype(cdt)

        o_rows = []
        for h in range(n_kv):
            q_h = q[:, h * group_w:h * group_w + _DH]
            for j in range(1, rep):
                q_h = jnp.where(row % rep == j,
                                q[:, h * group_w + j * _DH:h * group_w + (j + 1) * _DH], q_h)
            next_chunk()
            sc = lax.dot_general(q_h, k_v[h], (((1,), (1,)), ((), ())),
                                 preferred_element_type=f32) * sm_scale
            p = jnp.exp(sc - jnp.max(sc, axis=-1, keepdims=True))
            denom = jnp.sum(p, axis=-1, keepdims=True)
            next_chunk()
            o = jnp.dot(p.astype(cdt), v_v[h], preferred_element_type=f32) / denom
            o = o.astype(cdt)
            o_rows += [jnp.where(row == j, o, jnp.zeros_like(o)) for j in range(rep)]

        def up_proj(w_v):
            acc = jnp.zeros((_SUBLANES, d_ffn), f32)
            for s0, n in wgu_chunks:
                next_chunk()
                acc = acc + jnp.dot(x_rows[:, s0:s0 + n], w_v[pl.ds(s0, n), :],
                                    preferred_element_type=f32)
            return acc

        g = up_proj(wg_v)
        u = up_proj(wu_v)
        hid = (jax.nn.silu(g) * u).astype(cdt)

        hid_col = []
        for c0 in range(wd_mxu_total, d_ffn, _LANES):
            piece = hid[0:1, c0:c0 + _LANES].astype(f32) * gate_r
            hid_col.append(jnp.broadcast_to(piece, (_LANES, _LANES)).T)
        hid_col = jnp.concatenate(hid_col, axis=0)

        attn = jnp.zeros((_SUBLANES, d_model), f32)
        for s0, n in wo_chunks:
            next_chunk()
            lhs = jnp.concatenate(o_rows[s0 // _DH:(s0 + n) // _DH], axis=1)
            attn = attn + jnp.dot(lhs, wo_v[pl.ds(s0, n), :], preferred_element_type=f32)
        base = x + jnp.sum(attn, axis=0, keepdims=True) + (xn + xn * 0.0)

        y = jnp.zeros((_SUBLANES, d_model), f32)
        for s0, n in wd_chunks[:n_wd_mxu]:
            next_chunk()
            y = y + jnp.dot(hid[:, s0:s0 + n], wd_v[pl.ds(s0, n), :],
                            preferred_element_type=f32)
        row_d = lax.broadcasted_iota(jnp.int32, (_SUBLANES, d_model), 0)
        part = jnp.where(row_d == 0, base + y * gate_r, 0.0)
        for s0, n in wd_chunks[n_wd_mxu:]:
            next_chunk()
            w = wd_v[pl.ds(s0, n), :].astype(f32)
            hc = hid_col[s0 - wd_mxu_total:s0 - wd_mxu_total + n, :]
            prod = w * jnp.concatenate([hc] * (d_model // _LANES), axis=1)
            part = part + prod.reshape(n // _SUBLANES, _SUBLANES, d_model).sum(axis=0)
        assert waited[0] == started[0] == len(stream)

        out_v[0] = jnp.sum(part, axis=0, keepdims=True).astype(out_v.dtype)
        out_copy = pltpu.make_async_copy(out_v, out_hbm, out_sem.at[0])
        out_copy.start()
        out_copy.wait()

    def kernel_function(*refs):
        pl.run_scoped(lambda *sems: body(*refs, *sems), pltpu.SemaphoreType.DMA((_NUM_SEMS,)),
                      pltpu.SemaphoreType.DMA((2,)), pltpu.SemaphoreType.DMA((1,)))

    hbm = pl.BlockSpec(memory_space=pl.ANY)
    return pl.pallas_call(
        kernel_function,
        out_shape=jax.ShapeDtypeStruct(A_x.shape, cdt),
        in_specs=[hbm] * 9,
        out_specs=hbm,
        scratch_shapes=[
            pltpu.VMEM(A_x.shape, cdt),
            pltpu.VMEM(B_w_r.shape, B_w_r.dtype),
            pltpu.VMEM((n_kv, win, _DH), A_k_cache.dtype),
            pltpu.VMEM((n_kv, win, _DH), A_v_cache.dtype),
            pltpu.VMEM(A_wq.shape, A_wq.dtype),
            pltpu.VMEM(A_wo.shape, A_wo.dtype),
            pltpu.VMEM(B_w_gate.shape, B_w_gate.dtype),
            pltpu.VMEM(B_w_up.shape, B_w_up.dtype),
            pltpu.VMEM(B_w_down.shape, B_w_down.dtype),
            pltpu.VMEM(A_x.shape, cdt),
        ],
        compiler_params=pltpu.CompilerParams(vmem_limit_bytes=48 << 20),
        name="psum_swa_mod_decode",
    )(A_x, A_k_cache, A_v_cache, A_wq, A_wo, B_w_r, B_w_gate, B_w_up, B_w_down)
```

```python
import jax
import jax.numpy as jnp
from jax import lax
import jax.experimental.pallas as pl
import jax.experimental.pallas.tpu as pltpu

_HQ = 32
_DH = 128
_LN_EPS = 1e-5
_CHUNK_BYTES = 1 << 20
_PIECE_BYTES = 32 << 10
_AHEAD_BYTES = 4 << 20
_NUM_SEMS = 8
_PRIORITIES = (0, 1, 1)
_KV_SHIFT_BYTES = 4 << 10
_LANES = 128
_SUBLANES = 8


def _row_chunks(n_rows, rows_per_chunk):
    return [(s, min(rows_per_chunk, n_rows - s)) for s in range(0, n_rows, rows_per_chunk)]


@jax.jit
def pallas_parallel_sum__sliding_block_cached__moe_arch_mod__decode_kernel(
A_x: jax.Array,
    A_k_cache: jax.Array,
    A_v_cache: jax.Array,
    A_wq: jax.Array,
    A_wo: jax.Array,
    B_x: jax.Array,
    B_w_r: jax.Array,
    B_w_gate: jax.Array,
    B_w_up: jax.Array,
    B_w_down: jax.Array,
):
    del B_x
    f32 = jnp.float32
    cdt = A_x.dtype

    batch, s_q, d_model = A_x.shape
    _, n_kv, s_k, d_head = A_k_cache.shape
    d_ffn = B_w_gate.shape[1]
    assert batch == 1 and s_q == 1 and d_head == _DH and _HQ % n_kv == 0
    assert A_wq.shape == (d_model, _HQ * _DH) and A_wo.shape == (_HQ * _DH, d_model)
    assert B_w_gate.shape == B_w_up.shape == (d_model, d_ffn)
    assert B_w_down.shape == (d_ffn, d_model) and B_w_r.shape == (d_model,)
    win = min(4096, max(256, s_k // 4))
    rep = _HQ // n_kv
    assert rep <= _SUBLANES and _SUBLANES % rep == 0
    assert d_model % (2 * _LANES) == 0 and win % _LANES == 0 and d_ffn % _LANES == 0
    group_w = rep * _DH
    sm_scale = _DH ** -0.5
    itemsize = jnp.dtype(cdt).itemsize

    def rows_for(row_bytes):
        return max(_LANES, _CHUNK_BYTES // row_bytes // _LANES * _LANES)

    wq_chunks = _row_chunks(d_model, rows_for(_HQ * _DH * itemsize))
    wgu_chunks = _row_chunks(d_model, d_model // 2)
    wo_chunks = _row_chunks(_HQ * _DH, rows_for(d_model * itemsize))
    wd_vpu_rows = (128, 64, 32, 32)
    wd_mxu_total = d_ffn - sum(wd_vpu_rows)
    assert wd_mxu_total >= 0
    wd_mxu_rows = []
    left = wd_mxu_total
    while left > 0:
        step = min(left, 512 if left > 512 else 256)
        wd_mxu_rows.append(step)
        left -= step
    wd_chunks, s = [], 0
    for r in (*wd_mxu_rows, *wd_vpu_rows):
        wd_chunks.append((s, r))
        s += r
    n_wd_mxu = len(wd_mxu_rows)

    def body(x_hbm, k_hbm, v_hbm, wq_hbm, wo_hbm, wr_hbm, wg_hbm, wu_hbm, wd_hbm, out_hbm,
             x_v, wr_v, k_v, v_v, wq_v, wo_v, wg_v, wu_v, wd_v, out_v, sems, small_sems, out_sem):
        stream = []

        def enqueue(src, dst, n_rows, n_cols, shift_rows=0):
            row_bytes = n_cols * itemsize
            if 2 * row_bytes * _SUBLANES > 3 * _PIECE_BYTES:
                p_rows = _SUBLANES
                p_cols = max(_LANES, _PIECE_BYTES // (p_rows * itemsize) // _LANES * _LANES)
            else:
                p_rows = max(_SUBLANES, _PIECE_BYTES // row_bytes // _SUBLANES * _SUBLANES)
                p_cols = n_cols
            sem = sems.at[len(stream) % _NUM_SEMS]
            pieces = []
            cuts = [0, *range(p_rows - shift_rows, n_rows, p_rows), n_rows]
            for r0, r1 in zip(cuts[:-1], cuts[1:]):
                for c in range(0, n_cols, p_cols):
                    rows, cols = pl.ds(r0, r1 - r0), pl.ds(c, min(p_cols, n_cols - c))
                    if p_cols >= n_cols:
                        pieces.append(pltpu.make_async_copy(src.at[rows], dst.at[rows], sem))
                    else:
                        pieces.append(pltpu.make_async_copy(src.at[rows, cols], dst.at[rows, cols], sem))
            n_pat0 = _PRIORITIES.count(0)
            n0 = (len(pieces) * n_pat0 + len(_PRIORITIES) // 2) // len(_PRIORITIES)
            n0 = min(max(n0, 1), max(len(pieces) - 1, 1))
            todo = {0: pieces[:n0], 1: pieces[n0:]}
            issue, k = [], 0
            while todo[0] or todo[1]:
                prio = _PRIORITIES[k % len(_PRIORITIES)]
                k += 1
                if todo[prio]:
                    issue.append((todo[prio].pop(0), prio))
            stream.append((pltpu.make_async_copy(dst, dst, sem), issue, n_rows * row_bytes))

        for s0, n in wq_chunks:
            enqueue(wq_hbm.at[pl.ds(s0, n)], wq_v.at[pl.ds(s0, n)], n, _HQ * _DH)
        kv_shift = _KV_SHIFT_BYTES // (_DH * itemsize) // _SUBLANES * _SUBLANES
        for h in range(n_kv):
            enqueue(k_hbm.at[0, h, pl.ds(s_k - win, win)], k_v.at[h], win, _DH, kv_shift)
            enqueue(v_hbm.at[0, h, pl.ds(s_k - win, win)], v_v.at[h], win, _DH, kv_shift)
        for s0, n in wgu_chunks:
            enqueue(wg_hbm.at[pl.ds(s0, n)], wg_v.at[pl.ds(s0, n)], n, d_ffn)
        for s0, n in wgu_chunks:
            enqueue(wu_hbm.at[pl.ds(s0, n)], wu_v.at[pl.ds(s0, n)], n, d_ffn)
        for s0, n in wo_chunks:
            enqueue(wo_hbm.at[pl.ds(s0, n)], wo_v.at[pl.ds(s0, n)], n, d_model)
        for s0, n in wd_chunks:
            enqueue(wd_hbm.at[pl.ds(s0, n)], wd_v.at[pl.ds(s0, n)], n, d_model)
        started, waited = [0], [0]

        def top_up():
            while (started[0] < len(stream) and started[0] - waited[0] < _NUM_SEMS
                   and sum(c[2] for c in stream[waited[0]:started[0]]) < _AHEAD_BYTES):
                for copy, prio in stream[started[0]][1]:
                    copy.start(priority=prio)
                started[0] += 1

        def next_chunk():
            stream[waited[0]][0].wait()
            waited[0] += 1
            top_up()

        x_copy = pltpu.make_async_copy(x_hbm, x_v, small_sems.at[0])
        wr_copy = pltpu.make_async_copy(wr_hbm, wr_v, small_sems.at[1])
        x_copy.start()
        wr_copy.start()
        top_up()
        x_copy.wait()
        wr_copy.wait()

        row = lax.broadcasted_iota(jnp.int32, (_SUBLANES, _DH), 0)

        x = x_v[0].astype(f32)
        mean = jnp.mean(x, axis=-1, keepdims=True)
        xc = x - mean
        var = jnp.mean(xc * xc, axis=-1, keepdims=True)
        xn = xc / jnp.sqrt(var + _LN_EPS)
        xn_c = xn.astype(cdt)
        r = jnp.sum(xn_c.astype(f32) * wr_v[...].astype(f32).reshape(1, d_model),
                    axis=-1, keepdims=True)
        gate_r = jax.nn.sigmoid(r)
        x_rows = jnp.broadcast_to(xn_c, (_SUBLANES, d_model))

        q = jnp.zeros((_SUBLANES, _HQ * _DH), f32)
        for s0, n in wq_chunks:
            next_chunk()
            q = q + jnp.dot(x_rows[:, s0:s0 + n], wq_v[pl.ds(s0, n), :],
                            preferred_element_type=f32)
        q = q.astype(cdt)

        o_rows = []
        for h in range(n_kv):
            q_h = q[:, h * group_w:h * group_w + _DH]
            for j in range(1, rep):
                q_h = jnp.where(row % rep == j,
                                q[:, h * group_w + j * _DH:h * group_w + (j + 1) * _DH], q_h)
            next_chunk()
            sc = lax.dot_general(q_h, k_v[h], (((1,), (1,)), ((), ())),
                                 preferred_element_type=f32) * sm_scale
            p = jnp.exp(sc - jnp.max(sc, axis=-1, keepdims=True))
            denom = jnp.sum(p, axis=-1, keepdims=True)
            next_chunk()
            o = jnp.dot(p.astype(cdt), v_v[h], preferred_element_type=f32) / denom
            o = o.astype(cdt)
            o_rows += [jnp.where(row == j, o, jnp.zeros_like(o)) for j in range(rep)]

        def up_proj(w_v):
            acc = jnp.zeros((_SUBLANES, d_ffn), f32)
            for s0, n in wgu_chunks:
                next_chunk()
                acc = acc + jnp.dot(x_rows[:, s0:s0 + n], w_v[pl.ds(s0, n), :],
                                    preferred_element_type=f32)
            return acc

        g = up_proj(wg_v)
        u = up_proj(wu_v)
        hid = (jax.nn.silu(g) * u).astype(cdt)

        hid_col = []
        for c0 in range(wd_mxu_total, d_ffn, _LANES):
            piece = hid[0:1, c0:c0 + _LANES].astype(f32) * gate_r
            hid_col.append(jnp.broadcast_to(piece, (_LANES, _LANES)).T)
        hid_col = jnp.concatenate(hid_col, axis=0)

        attn = jnp.zeros((_SUBLANES, d_model), f32)
        for s0, n in wo_chunks:
            next_chunk()
            lhs = jnp.concatenate(o_rows[s0 // _DH:(s0 + n) // _DH], axis=1)
            attn = attn + jnp.dot(lhs, wo_v[pl.ds(s0, n), :], preferred_element_type=f32)
        base = x + jnp.sum(attn, axis=0, keepdims=True) + (xn + xn * 0.0)

        y = jnp.zeros((_SUBLANES, d_model), f32)
        for s0, n in wd_chunks[:n_wd_mxu]:
            next_chunk()
            y = y + jnp.dot(hid[:, s0:s0 + n], wd_v[pl.ds(s0, n), :],
                            preferred_element_type=f32)
        row_d = lax.broadcasted_iota(jnp.int32, (_SUBLANES, d_model), 0)
        part = jnp.where(row_d == 0, base + y * gate_r, 0.0)
        for s0, n in wd_chunks[n_wd_mxu:]:
            next_chunk()
            w = wd_v[pl.ds(s0, n), :].astype(f32)
            hc = hid_col[s0 - wd_mxu_total:s0 - wd_mxu_total + n, :]
            prod = w * jnp.concatenate([hc] * (d_model // _LANES), axis=1)
            part = part + prod.reshape(n // _SUBLANES, _SUBLANES, d_model).sum(axis=0)
        assert waited[0] == started[0] == len(stream)

        out_v[0] = jnp.sum(part, axis=0, keepdims=True).astype(out_v.dtype)
        out_copy = pltpu.make_async_copy(out_v, out_hbm, out_sem.at[0])
        out_copy.start()
        out_copy.wait()

    def kernel_function(*refs):
        pl.run_scoped(lambda *sems: body(*refs, *sems), pltpu.SemaphoreType.DMA((_NUM_SEMS,)),
                      pltpu.SemaphoreType.DMA((2,)), pltpu.SemaphoreType.DMA((1,)))

    hbm = pl.BlockSpec(memory_space=pl.ANY)
    return pl.pallas_call(
        kernel_function,
        out_shape=jax.ShapeDtypeStruct(A_x.shape, cdt),
        in_specs=[hbm] * 9,
        out_specs=hbm,
        scratch_shapes=[
            pltpu.VMEM(A_x.shape, cdt),
            pltpu.VMEM(B_w_r.shape, B_w_r.dtype),
            pltpu.VMEM((n_kv, win, _DH), A_k_cache.dtype),
            pltpu.VMEM((n_kv, win, _DH), A_v_cache.dtype),
            pltpu.VMEM(A_wq.shape, A_wq.dtype),
            pltpu.VMEM(A_wo.shape, A_wo.dtype),
            pltpu.VMEM(B_w_gate.shape, B_w_gate.dtype),
            pltpu.VMEM(B_w_up.shape, B_w_up.dtype),
            pltpu.VMEM(B_w_down.shape, B_w_down.dtype),
            pltpu.VMEM(A_x.shape, cdt),
        ],
        compiler_params=pltpu.CompilerParams(vmem_limit_bytes=48 << 20),
        name="psum_swa_mod_decode",
    )(A_x, A_k_cache, A_v_cache, A_wq, A_wo, B_w_r, B_w_gate, B_w_up, B_w_down)
```

```python
import jax
import jax.numpy as jnp
from jax import lax
import jax.experimental.pallas as pl
import jax.experimental.pallas.tpu as pltpu

_HQ = 32
_DH = 128
_LN_EPS = 1e-5
_CHUNK_BYTES = 1 << 20
_PIECE_BYTES = 32 << 10
_AHEAD_BYTES = 4 << 20
_NUM_SEMS = 8
_PRIORITIES = (0, 1, 1)
_KV_SHIFT_BYTES = 4 << 10
_LANES = 128
_SUBLANES = 8


def _row_chunks(n_rows, rows_per_chunk):
    return [(s, min(rows_per_chunk, n_rows - s)) for s in range(0, n_rows, rows_per_chunk)]


@jax.jit
def pallas_parallel_sum__sliding_block_cached__moe_arch_mod__decode_kernel(
A_x: jax.Array,
    A_k_cache: jax.Array,
    A_v_cache: jax.Array,
    A_wq: jax.Array,
    A_wo: jax.Array,
    B_x: jax.Array,
    B_w_r: jax.Array,
    B_w_gate: jax.Array,
    B_w_up: jax.Array,
    B_w_down: jax.Array,
):
    del B_x
    f32 = jnp.float32
    cdt = A_x.dtype

    batch, s_q, d_model = A_x.shape
    _, n_kv, s_k, d_head = A_k_cache.shape
    d_ffn = B_w_gate.shape[1]
    assert batch == 1 and s_q == 1 and d_head == _DH and _HQ % n_kv == 0
    assert A_wq.shape == (d_model, _HQ * _DH) and A_wo.shape == (_HQ * _DH, d_model)
    assert B_w_gate.shape == B_w_up.shape == (d_model, d_ffn)
    assert B_w_down.shape == (d_ffn, d_model) and B_w_r.shape == (d_model,)
    win = min(4096, max(256, s_k // 4))
    rep = _HQ // n_kv
    assert rep <= _SUBLANES and _SUBLANES % rep == 0
    assert d_model % (2 * _LANES) == 0 and win % _LANES == 0 and d_ffn % _LANES == 0
    group_w = rep * _DH
    sm_scale = _DH ** -0.5
    itemsize = jnp.dtype(cdt).itemsize

    def rows_for(row_bytes):
        return max(_LANES, _CHUNK_BYTES // row_bytes // _LANES * _LANES)

    wq_chunks = _row_chunks(d_model, rows_for(_HQ * _DH * itemsize))
    wgu_chunks = _row_chunks(d_model, d_model // 2)
    wo_chunks = _row_chunks(_HQ * _DH, rows_for(d_model * itemsize))
    wd_vpu_rows = (128, 64, 32, 32)
    wd_mxu_total = d_ffn - sum(wd_vpu_rows)
    assert wd_mxu_total >= 0
    wd_mxu_rows = []
    left = wd_mxu_total
    while left > 0:
        step = min(left, 512 if left > 512 else 256)
        wd_mxu_rows.append(step)
        left -= step
    wd_chunks, s = [], 0
    for r in (*wd_mxu_rows, *wd_vpu_rows):
        wd_chunks.append((s, r))
        s += r
    n_wd_mxu = len(wd_mxu_rows)

    def body(x_hbm, k_hbm, v_hbm, wq_hbm, wo_hbm, wr_hbm, wg_hbm, wu_hbm, wd_hbm, out_hbm,
             x_v, wr_v, k_v, v_v, wq_v, wo_v, wg_v, wu_v, wd_v, out_v, sems, small_sems, out_sem):
        stream = []

        def enqueue(src, dst, n_rows, n_cols, shift_rows=0, one_queue=False):
            row_bytes = n_cols * itemsize
            if 2 * row_bytes * _SUBLANES > 3 * _PIECE_BYTES:
                p_rows = _SUBLANES
                p_cols = max(_LANES, _PIECE_BYTES // (p_rows * itemsize) // _LANES * _LANES)
            else:
                p_rows = max(_SUBLANES, _PIECE_BYTES // row_bytes // _SUBLANES * _SUBLANES)
                p_cols = n_cols
            sem = sems.at[len(stream) % _NUM_SEMS]
            pieces = []
            cuts = [0, *range(p_rows - shift_rows, n_rows, p_rows), n_rows]
            for r0, r1 in zip(cuts[:-1], cuts[1:]):
                for c in range(0, n_cols, p_cols):
                    rows, cols = pl.ds(r0, r1 - r0), pl.ds(c, min(p_cols, n_cols - c))
                    if p_cols >= n_cols:
                        pieces.append(pltpu.make_async_copy(src.at[rows], dst.at[rows], sem))
                    else:
                        pieces.append(pltpu.make_async_copy(src.at[rows, cols], dst.at[rows, cols], sem))
            n_pat0 = _PRIORITIES.count(0)
            n0 = (len(pieces) * n_pat0 + len(_PRIORITIES) // 2) // len(_PRIORITIES)
            n0 = 0 if one_queue else min(max(n0, 1), max(len(pieces) - 1, 1))
            todo = {0: pieces[:n0], 1: pieces[n0:]}
            issue, k = [], 0
            while todo[0] or todo[1]:
                prio = _PRIORITIES[k % len(_PRIORITIES)]
                k += 1
                if todo[prio]:
                    issue.append((todo[prio].pop(0), prio))
            stream.append((pltpu.make_async_copy(dst, dst, sem), issue, n_rows * row_bytes))

        for s0, n in wq_chunks:
            enqueue(wq_hbm.at[pl.ds(s0, n)], wq_v.at[pl.ds(s0, n)], n, _HQ * _DH)
        kv_shift = _KV_SHIFT_BYTES // (_DH * itemsize) // _SUBLANES * _SUBLANES
        for h in range(n_kv):
            enqueue(k_hbm.at[0, h, pl.ds(s_k - win, win)], k_v.at[h], win, _DH, kv_shift)
            enqueue(v_hbm.at[0, h, pl.ds(s_k - win, win)], v_v.at[h], win, _DH, kv_shift)
        for s0, n in wgu_chunks:
            enqueue(wg_hbm.at[pl.ds(s0, n)], wg_v.at[pl.ds(s0, n)], n, d_ffn)
        for s0, n in wgu_chunks:
            enqueue(wu_hbm.at[pl.ds(s0, n)], wu_v.at[pl.ds(s0, n)], n, d_ffn)
        for s0, n in wo_chunks:
            enqueue(wo_hbm.at[pl.ds(s0, n)], wo_v.at[pl.ds(s0, n)], n, d_model)
        for i, (s0, n) in enumerate(wd_chunks):
            enqueue(wd_hbm.at[pl.ds(s0, n)], wd_v.at[pl.ds(s0, n)], n, d_model,
                    one_queue=i >= n_wd_mxu - 1)
        started, waited = [0], [0]

        def top_up():
            while (started[0] < len(stream) and started[0] - waited[0] < _NUM_SEMS
                   and sum(c[2] for c in stream[waited[0]:started[0]]) < _AHEAD_BYTES):
                for copy, prio in stream[started[0]][1]:
                    copy.start(priority=prio)
                started[0] += 1

        def next_chunk():
            stream[waited[0]][0].wait()
            waited[0] += 1
            top_up()

        x_copy = pltpu.make_async_copy(x_hbm, x_v, small_sems.at[0])
        wr_copy = pltpu.make_async_copy(wr_hbm, wr_v, small_sems.at[1])
        x_copy.start()
        wr_copy.start()
        top_up()
        x_copy.wait()
        wr_copy.wait()

        row = lax.broadcasted_iota(jnp.int32, (_SUBLANES, _DH), 0)

        x = x_v[0].astype(f32)
        mean = jnp.mean(x, axis=-1, keepdims=True)
        xc = x - mean
        var = jnp.mean(xc * xc, axis=-1, keepdims=True)
        xn = xc / jnp.sqrt(var + _LN_EPS)
        xn_c = xn.astype(cdt)
        r = jnp.sum(xn_c.astype(f32) * wr_v[...].astype(f32).reshape(1, d_model),
                    axis=-1, keepdims=True)
        gate_r = jax.nn.sigmoid(r)
        x_rows = jnp.broadcast_to(xn_c, (_SUBLANES, d_model))

        q = jnp.zeros((_SUBLANES, _HQ * _DH), f32)
        for s0, n in wq_chunks:
            next_chunk()
            q = q + jnp.dot(x_rows[:, s0:s0 + n], wq_v[pl.ds(s0, n), :],
                            preferred_element_type=f32)
        q = q.astype(cdt)

        o_rows = []
        for h in range(n_kv):
            q_h = q[:, h * group_w:h * group_w + _DH]
            for j in range(1, rep):
                q_h = jnp.where(row % rep == j,
                                q[:, h * group_w + j * _DH:h * group_w + (j + 1) * _DH], q_h)
            next_chunk()
            sc = lax.dot_general(q_h, k_v[h], (((1,), (1,)), ((), ())),
                                 preferred_element_type=f32) * sm_scale
            p = jnp.exp(sc - jnp.max(sc, axis=-1, keepdims=True))
            denom = jnp.sum(p, axis=-1, keepdims=True)
            next_chunk()
            o = jnp.dot(p.astype(cdt), v_v[h], preferred_element_type=f32) / denom
            o = o.astype(cdt)
            o_rows += [jnp.where(row == j, o, jnp.zeros_like(o)) for j in range(rep)]

        def up_proj(w_v):
            acc = jnp.zeros((_SUBLANES, d_ffn), f32)
            for s0, n in wgu_chunks:
                next_chunk()
                acc = acc + jnp.dot(x_rows[:, s0:s0 + n], w_v[pl.ds(s0, n), :],
                                    preferred_element_type=f32)
            return acc

        g = up_proj(wg_v)
        u = up_proj(wu_v)
        hid = (jax.nn.silu(g) * u).astype(cdt)

        hid_col = []
        for c0 in range(wd_mxu_total, d_ffn, _LANES):
            piece = hid[0:1, c0:c0 + _LANES].astype(f32) * gate_r
            hid_col.append(jnp.broadcast_to(piece, (_LANES, _LANES)).T)
        hid_col = jnp.concatenate(hid_col, axis=0)

        attn = jnp.zeros((_SUBLANES, d_model), f32)
        for s0, n in wo_chunks:
            next_chunk()
            lhs = jnp.concatenate(o_rows[s0 // _DH:(s0 + n) // _DH], axis=1)
            attn = attn + jnp.dot(lhs, wo_v[pl.ds(s0, n), :], preferred_element_type=f32)
        base = x + jnp.sum(attn, axis=0, keepdims=True) + (xn + xn * 0.0)

        y = jnp.zeros((_SUBLANES, d_model), f32)
        for s0, n in wd_chunks[:n_wd_mxu]:
            next_chunk()
            y = y + jnp.dot(hid[:, s0:s0 + n], wd_v[pl.ds(s0, n), :],
                            preferred_element_type=f32)
        row_d = lax.broadcasted_iota(jnp.int32, (_SUBLANES, d_model), 0)
        part = jnp.where(row_d == 0, base + y * gate_r, 0.0)
        for s0, n in wd_chunks[n_wd_mxu:]:
            next_chunk()
            w = wd_v[pl.ds(s0, n), :].astype(f32)
            hc = hid_col[s0 - wd_mxu_total:s0 - wd_mxu_total + n, :]
            prod = w * jnp.concatenate([hc] * (d_model // _LANES), axis=1)
            part = part + prod.reshape(n // _SUBLANES, _SUBLANES, d_model).sum(axis=0)
        assert waited[0] == started[0] == len(stream)

        out_v[0] = jnp.sum(part, axis=0, keepdims=True).astype(out_v.dtype)
        out_copy = pltpu.make_async_copy(out_v, out_hbm, out_sem.at[0])
        out_copy.start()
        out_copy.wait()

    def kernel_function(*refs):
        pl.run_scoped(lambda *sems: body(*refs, *sems), pltpu.SemaphoreType.DMA((_NUM_SEMS,)),
                      pltpu.SemaphoreType.DMA((2,)), pltpu.SemaphoreType.DMA((1,)))

    hbm = pl.BlockSpec(memory_space=pl.ANY)
    return pl.pallas_call(
        kernel_function,
        out_shape=jax.ShapeDtypeStruct(A_x.shape, cdt),
        in_specs=[hbm] * 9,
        out_specs=hbm,
        scratch_shapes=[
            pltpu.VMEM(A_x.shape, cdt),
            pltpu.VMEM(B_w_r.shape, B_w_r.dtype),
            pltpu.VMEM((n_kv, win, _DH), A_k_cache.dtype),
            pltpu.VMEM((n_kv, win, _DH), A_v_cache.dtype),
            pltpu.VMEM(A_wq.shape, A_wq.dtype),
            pltpu.VMEM(A_wo.shape, A_wo.dtype),
            pltpu.VMEM(B_w_gate.shape, B_w_gate.dtype),
            pltpu.VMEM(B_w_up.shape, B_w_up.dtype),
            pltpu.VMEM(B_w_down.shape, B_w_down.dtype),
            pltpu.VMEM(A_x.shape, cdt),
        ],
        compiler_params=pltpu.CompilerParams(vmem_limit_bytes=48 << 20),
        name="psum_swa_mod_decode",
    )(A_x, A_k_cache, A_v_cache, A_wq, A_wo, B_w_r, B_w_gate, B_w_up, B_w_down)
```

```python
import jax
import jax.numpy as jnp
from jax import lax
import jax.experimental.pallas as pl
import jax.experimental.pallas.tpu as pltpu

_HQ = 32
_DH = 128
_LN_EPS = 1e-5
_LANES = 128
_SUBLANES = 8

_CHUNK_BYTES = 1 << 20
_PIECE_BYTES = 32 << 10
_SLOTS = 4
_AHEAD = 96
_LAG = 70


def _row_chunks(n_rows, rows_per_chunk):
    return [(s, min(rows_per_chunk, n_rows - s)) for s in range(0, n_rows, rows_per_chunk)]


def _ramp_chunks(n_rows, n_chunks, unit):
    units = n_rows // unit
    total = n_chunks * (n_chunks + 1) // 2
    sizes = [max(1, units * (i + 1) // total) for i in range(n_chunks)]
    i = n_chunks - 1
    while sum(sizes) < units:
        sizes[i] += 1
        i = i - 1 if i > n_chunks // 2 else n_chunks - 1
    while sum(sizes) > units:
        sizes[sizes.index(max(sizes))] -= 1
    out, s = [], 0
    for n in sizes:
        if n:
            out.append((s, n * unit))
            s += n * unit
    return out


@jax.jit
def pallas_parallel_sum__sliding_block_cached__moe_arch_mod__decode_kernel(
A_x: jax.Array,
    A_k_cache: jax.Array,
    A_v_cache: jax.Array,
    A_wq: jax.Array,
    A_wo: jax.Array,
    B_x: jax.Array,
    B_w_r: jax.Array,
    B_w_gate: jax.Array,
    B_w_up: jax.Array,
    B_w_down: jax.Array,
):
    del B_x
    f32 = jnp.float32
    cdt = A_x.dtype

    batch, s_q, d_model = A_x.shape
    _, n_kv, s_k, d_head = A_k_cache.shape
    d_ffn = B_w_gate.shape[1]
    d_q = _HQ * _DH
    assert batch == 1 and s_q == 1 and d_head == _DH and _HQ % n_kv == 0
    assert A_wq.shape == (d_model, d_q) and A_wo.shape == (d_q, d_model)
    assert B_w_gate.shape == B_w_up.shape == (d_model, d_ffn)
    assert B_w_down.shape == (d_ffn, d_model) and B_w_r.shape == (d_model,)
    win = min(4096, max(256, s_k // 4))
    rep = _HQ // n_kv
    assert rep <= _SUBLANES and _SUBLANES % rep == 0
    assert d_model % (2 * _LANES) == 0 and win % _LANES == 0 and d_ffn % _LANES == 0
    group_w = rep * _DH
    sm_scale = _DH ** -0.5
    itemsize = jnp.dtype(cdt).itemsize

    wq_chunks = _ramp_chunks(d_model, 2 * _SLOTS, _SUBLANES)
    wgu_chunks = _row_chunks(d_model, d_model // 2)
    wo_rows = max(group_w, _CHUNK_BYTES // (d_model * itemsize) // group_w * group_w)
    wo_chunks = _row_chunks(d_q, wo_rows)
    wd_vpu_rows = (128, 64, 32, 32)
    wd_mxu_total = d_ffn - sum(wd_vpu_rows)
    assert wd_mxu_total > 0
    wd_mxu_rows, left = [], wd_mxu_total
    while left > 0:
        step = min(left, 512 if left > 512 else 256)
        wd_mxu_rows.append(step)
        left -= step
    wd_chunks, s = [], 0
    for r in (*wd_mxu_rows, *wd_vpu_rows):
        wd_chunks.append((s, r))
        s += r
    n_wd_early = len(wd_mxu_rows) - 1
    n_chunks = len(wq_chunks) + 2 * n_kv + 2 * len(wgu_chunks) + len(wo_chunks) + len(wd_chunks)

    def body(x_hbm, k_hbm, v_hbm, wq_hbm, wo_hbm, wr_hbm, wg_hbm, wu_hbm, wd_hbm, out_hbm,
             x_v, wr_v, k_v, v_v, wq_v, wo_v, wg_v, wu_v, wd_v, out_v, sems, small_sems, out_sem):
        chunks = {}

        def add_chunk(name, src, dst, n_rows, n_cols):
            row_bytes = n_cols * itemsize
            if 2 * row_bytes * _SUBLANES > 3 * _PIECE_BYTES:
                p_rows = _SUBLANES
                p_cols = max(_LANES, _PIECE_BYTES // (p_rows * itemsize) // _LANES * _LANES)
            else:
                p_rows = max(_SUBLANES, _PIECE_BYTES // row_bytes // _SUBLANES * _SUBLANES)
                p_cols = n_cols
            pieces = []
            for r in range(0, n_rows, p_rows):
                for c in range(0, n_cols, p_cols):
                    rows, cols = pl.ds(r, min(p_rows, n_rows - r)), pl.ds(c, min(p_cols, n_cols - c))
                    if p_cols >= n_cols:
                        pieces.append((src.at[rows], dst.at[rows]))
                    else:
                        pieces.append((src.at[rows, cols], dst.at[rows, cols]))
            chunks[name] = (dst, pieces)
            return name

        def add_rows(prefix, hbm, vmem, ranges, n_cols):
            return [add_chunk(f"{prefix}{i}", hbm.at[pl.ds(s0, n)], vmem.at[pl.ds(s0, n)], n, n_cols)
                    for i, (s0, n) in enumerate(ranges)]

        c_wq = add_rows("q", wq_hbm, wq_v, wq_chunks, d_q)
        c_k = [add_chunk(f"k{h}", k_hbm.at[0, h, pl.ds(s_k - win, win)], k_v.at[h], win, _DH)
               for h in range(n_kv)]
        c_v = [add_chunk(f"v{h}", v_hbm.at[0, h, pl.ds(s_k - win, win)], v_v.at[h], win, _DH)
               for h in range(n_kv)]
        c_wg = add_rows("g", wg_hbm, wg_v, wgu_chunks, d_ffn)
        c_wu = add_rows("u", wu_hbm, wu_v, wgu_chunks, d_ffn)
        c_wo = add_rows("o", wo_hbm, wo_v, wo_chunks, d_model)
        c_wd = add_rows("d", wd_hbm, wd_v, wd_chunks, d_model)
        c_wd_early, c_tail = c_wd[:n_wd_early], c_wd[n_wd_early:]

        n_wo0 = len(c_wo) // 2
        pending = (
            c_wq[0::2] + c_wg + c_k + c_wd_early[0::2] + c_wo[:n_wo0],
            c_wq[1::2] + c_wu + c_v + c_wd_early[1::2] + c_wo[n_wo0:],
        )
        slots = ([None] * _SLOTS, [None] * _SLOTS)
        cursor = dict.fromkeys(chunks, 0)
        issue = []
        while any(pending) or any(c is not None for q_slots in slots for c in q_slots):
            for queue in (0, 1):
                for s in range(_SLOTS):
                    if slots[queue][s] is None and pending[queue]:
                        slots[queue][s] = pending[queue].pop(0)
            for s in range(_SLOTS):
                for queue in (0, 1):
                    c = slots[queue][s]
                    if c is not None:
                        issue.append((c, cursor[c], queue))
                        cursor[c] += 1
                        if cursor[c] == len(chunks[c][1]):
                            slots[queue][s] = None
        for c in c_tail:
            issue += [(c, j, 1) for j in range(len(chunks[c][1]))]
        last_pos = {c: pos for pos, (c, _, _) in enumerate(issue)}
        landing = {c: last_pos[c] + (_LAG if queue else 0) for c, _, queue in issue}

        assert len(chunks) == n_chunks
        sem_of = {c: sems.at[i] for i, c in enumerate(chunks)}
        issued, landed = [0], set()

        def issue_upto(n):
            while issued[0] < min(n, len(issue)):
                c, j, queue = issue[issued[0]]
                src, dst = chunks[c][1][j]
                pltpu.make_async_copy(src, dst, sem_of[c]).start(priority=queue)
                issued[0] += 1

        def need(c):
            if c not in landed:
                issue_upto(last_pos[c] + 1 + _AHEAD)
                dst = chunks[c][0]
                pltpu.make_async_copy(dst, dst, sem_of[c]).wait()
                landed.add(c)

        x_copy = pltpu.make_async_copy(x_hbm, x_v, small_sems.at[0])
        wr_copy = pltpu.make_async_copy(wr_hbm, wr_v, small_sems.at[1])
        x_copy.start()
        wr_copy.start()
        issue_upto(last_pos[c_wq[0]] + 1 + _AHEAD)
        x_copy.wait()
        wr_copy.wait()

        row = lax.broadcasted_iota(jnp.int32, (_SUBLANES, _DH), 0)

        x = x_v[0].astype(f32)
        mean = jnp.mean(x, axis=-1, keepdims=True)
        xc = x - mean
        var = jnp.mean(xc * xc, axis=-1, keepdims=True)
        xn = xc / jnp.sqrt(var + _LN_EPS)
        xn_c = xn.astype(cdt)
        r = jnp.sum(xn_c.astype(f32) * wr_v[...].astype(f32).reshape(1, d_model),
                    axis=-1, keepdims=True)
        gate_r = jax.nn.sigmoid(r)
        x_rows = jnp.broadcast_to(xn_c, (_SUBLANES, d_model))

        val = {
            "g": jnp.zeros((_SUBLANES, d_ffn), f32),
            "u": jnp.zeros((_SUBLANES, d_ffn), f32),
            "attn": jnp.zeros((_SUBLANES, d_model), f32),
            "y": jnp.zeros((_SUBLANES, d_model), f32),
        }

        def q_proj():
            q = jnp.zeros((_SUBLANES, d_q), f32)
            for s0 in range(0, d_model, _LANES):
                for c, (c0, n) in zip(c_wq, wq_chunks):
                    if c0 < s0 + _LANES and c0 + n > s0:
                        need(c)
                q = q + jnp.dot(x_rows[:, s0:s0 + _LANES], wq_v[pl.ds(s0, _LANES), :],
                                preferred_element_type=f32)
            val["q"] = q.astype(cdt)

        def scores(h):
            q = val["q"]
            q_h = q[:, h * group_w:h * group_w + _DH]
            for j in range(1, rep):
                q_h = jnp.where(row % rep == j,
                                q[:, h * group_w + j * _DH:h * group_w + (j + 1) * _DH], q_h)
            need(c_k[h])
            sc = lax.dot_general(q_h, k_v[h], (((1,), (1,)), ((), ())),
                                 preferred_element_type=f32) * sm_scale
            p = jnp.exp(sc - jnp.max(sc, axis=-1, keepdims=True))
            val["p", h] = (p.astype(cdt), jnp.sum(p, axis=-1, keepdims=True))

        def values(h):
            need(c_v[h])
            p, denom = val.pop(("p", h))
            o = (jnp.dot(p, v_v[h], preferred_element_type=f32) / denom).astype(cdt)
            val["o", h] = [jnp.where(row == j, o, jnp.zeros_like(o)) for j in range(rep)]

        def up_proj(kind, i):
            names, w_v = (c_wg, wg_v) if kind == "g" else (c_wu, wu_v)
            s0, n = wgu_chunks[i]
            need(names[i])
            val[kind] = val[kind] + jnp.dot(x_rows[:, s0:s0 + n], w_v[pl.ds(s0, n), :],
                                            preferred_element_type=f32)

        def hidden():
            hid = (jax.nn.silu(val.pop("g")) * val.pop("u")).astype(cdt)
            val["hid"] = hid
            cols = []
            for c0 in range(wd_mxu_total, d_ffn, _LANES):
                piece = hid[0:1, c0:c0 + _LANES].astype(f32) * gate_r
                cols.append(jnp.broadcast_to(piece, (_LANES, _LANES)).T)
            val["hid_col"] = jnp.concatenate(cols, axis=0)

        def out_proj(i):
            s0, n = wo_chunks[i]
            need(c_wo[i])
            lhs = jnp.concatenate(
                [blk for h in range(s0 // group_w, (s0 + n) // group_w) for blk in val.pop(("o", h))],
                axis=1)
            val["attn"] = val["attn"] + jnp.dot(lhs, wo_v[pl.ds(s0, n), :],
                                                preferred_element_type=f32)

        def down_proj(i):
            s0, n = wd_chunks[i]
            need(c_wd[i])
            val["y"] = val["y"] + jnp.dot(val["hid"][:, s0:s0 + n], wd_v[pl.ds(s0, n), :],
                                          preferred_element_type=f32)

        steps = {"Q": (q_proj, max(landing[c] for c in c_wq), ())}
        for h in range(n_kv):
            steps[c_k[h]] = (lambda h=h: scores(h), landing[c_k[h]], ("Q",))
            steps[c_v[h]] = (lambda h=h: values(h), landing[c_v[h]], (c_k[h],))
        for kind, names in (("g", c_wg), ("u", c_wu)):
            for i, c in enumerate(names):
                steps[c] = (lambda kind=kind, i=i: up_proj(kind, i), landing[c], ())
        steps["H"] = (hidden, 0, (*c_wg, *c_wu))
        for i, (s0, n) in enumerate(wo_chunks):
            steps[c_wo[i]] = (lambda i=i: out_proj(i), landing[c_wo[i]],
                              tuple(c_v[s0 // group_w:(s0 + n) // group_w]))
        for i, c in enumerate(c_wd_early):
            steps[c] = (lambda i=i: down_proj(i), landing[c], ("H",))
        while steps:
            ready = [n for n, (_, _, deps) in steps.items() if not any(d in steps for d in deps)]
            steps.pop(min(ready, key=lambda n: steps[n][1]))[0]()

        base = x + jnp.sum(val["attn"], axis=0, keepdims=True) + (xn + xn * 0.0)

        down_proj(n_wd_early)
        row_d = lax.broadcasted_iota(jnp.int32, (_SUBLANES, d_model), 0)
        part = jnp.where(row_d == 0, base + val["y"] * gate_r, 0.0)
        for i in range(n_wd_early + 1, len(wd_chunks)):
            s0, n = wd_chunks[i]
            need(c_wd[i])
            w = wd_v[pl.ds(s0, n), :].astype(f32)
            hc = val["hid_col"][s0 - wd_mxu_total:s0 - wd_mxu_total + n, :]
            prod = w * jnp.concatenate([hc] * (d_model // _LANES), axis=1)
            part = part + prod.reshape(n // _SUBLANES, _SUBLANES, d_model).sum(axis=0)
        assert issued[0] == len(issue) and landed == set(chunks)

        out_v[0] = jnp.sum(part, axis=0, keepdims=True).astype(out_v.dtype)
        out_copy = pltpu.make_async_copy(out_v, out_hbm, out_sem.at[0])
        out_copy.start()
        out_copy.wait()

    def kernel_function(*refs):
        pl.run_scoped(lambda *sems: body(*refs, *sems), pltpu.SemaphoreType.DMA((n_chunks,)),
                      pltpu.SemaphoreType.DMA((2,)), pltpu.SemaphoreType.DMA((1,)))

    hbm = pl.BlockSpec(memory_space=pl.ANY)
    return pl.pallas_call(
        kernel_function,
        out_shape=jax.ShapeDtypeStruct(A_x.shape, cdt),
        in_specs=[hbm] * 9,
        out_specs=hbm,
        scratch_shapes=[
            pltpu.VMEM(A_x.shape, cdt),
            pltpu.VMEM(B_w_r.shape, B_w_r.dtype),
            pltpu.VMEM((n_kv, win, _DH), A_k_cache.dtype),
            pltpu.VMEM((n_kv, win, _DH), A_v_cache.dtype),
            pltpu.VMEM(A_wq.shape, A_wq.dtype),
            pltpu.VMEM(A_wo.shape, A_wo.dtype),
            pltpu.VMEM(B_w_gate.shape, B_w_gate.dtype),
            pltpu.VMEM(B_w_up.shape, B_w_up.dtype),
            pltpu.VMEM(B_w_down.shape, B_w_down.dtype),
            pltpu.VMEM(A_x.shape, cdt),
        ],
        compiler_params=pltpu.CompilerParams(vmem_limit_bytes=48 << 20),
        name="psum_swa_mod_decode",
    )(A_x, A_k_cache, A_v_cache, A_wq, A_wo, B_w_r, B_w_gate, B_w_up, B_w_down)
```
